```python
import jax
import jax.numpy as jnp

def _softmax(x, axis=-1):
    return jax.nn.softmax(x, axis=axis)
def _gelu(x):
    return jax.nn.gelu(x, approximate=True)
def _silu(x):
    return jax.nn.silu(x)
def _sigmoid(x):
    return jax.nn.sigmoid(x)
def _layernorm(x, axis=-1, eps=1e-5):
    m = jnp.mean(x, axis=axis, keepdims=True)
    v = jnp.var(x, axis=axis, keepdims=True)
    return (x - m) / jnp.sqrt(v + eps)
def _scatter_add(tgt, idx, src, axis=0):
    return tgt.at[idx].add(src)
def _segment_sum(src, seg, n):
    return jax.ops.segment_sum(src, seg, n)
class _Rng:
    def __init__(self, key):
        self._k = key
    def _next(self):
        self._k, sub = jax.random.split(self._k)
        return sub
    def normal(self, shape):
        return jax.random.normal(self._next(), shape, dtype=jnp.bfloat16)
    def randint(self, lo, hi, shape):
        return jax.random.randint(self._next(), shape, lo, hi, dtype=jnp.int32)
    def uniform(self, shape, lo=0.0, hi=1.0):
        return jax.random.uniform(self._next(), shape, jnp.bfloat16, lo, hi)
    def permutation(self, n):
        return jax.random.permutation(self._next(), n)


kernel_name = 'sequential_preLN__mha_block_cached__moe_arch_mod__decode'

def setup_inputs():
    _rng = _Rng(jax.random.key(int.from_bytes(__import__("os").urandom(4), "little")))
    _w = (lambda a: (lambda t: t.astype(jnp.bfloat16) if jnp.issubdtype(t.dtype, jnp.floating) else t)(jnp.asarray(a)))
    def _A_setup():
        B, Sq, D = 4, 1, 640
        H, Sk, Dh = 32, 8192, 192
        return {
            "x": _w((lambda *s: _rng.normal(s) * 0.05)(B, Sq, D)),
            "k_cache": _w((lambda *s: _rng.normal(s) * 0.05)(B, H, Sk, Dh)),
            "v_cache": _w((lambda *s: _rng.normal(s) * 0.05)(B, H, Sk, Dh)),
            "wq": _w((lambda *s: _rng.normal(s) * 0.05)(D, H * Dh) * (D ** -0.5)),
            "wo": _w((lambda *s: _rng.normal(s) * 0.05)(H * Dh, D) * ((H * Dh) ** -0.5)),
        }
    _A_in = _A_setup()

    def _B_setup():
        B, S, D, F, C = 4, 1, 640, 1536, 1
        return {
            "x": _w((lambda *s: _rng.normal(s) * 0.05)(B, S, D)),
            "w_r": _w((lambda *s: _rng.normal(s) * 0.05)(D)),
            "w_gate": _w((lambda *s: _rng.normal(s) * 0.05)(D, F)),
            "w_up": _w((lambda *s: _rng.normal(s) * 0.05)(D, F)),
            "w_down": _w((lambda *s: _rng.normal(s) * 0.05)(F, D)),
        }
    _B_in = _B_setup()

    return {
        "A_x": _A_in["x"],
        "A_k_cache": _A_in["k_cache"],
        "A_v_cache": _A_in["v_cache"],
        "A_wq": _A_in["wq"],
        "A_wo": _A_in["wo"],
        "B_x": _B_in["x"],
        "B_w_r": _B_in["w_r"],
        "B_w_gate": _B_in["w_gate"],
        "B_w_up": _B_in["w_up"],
        "B_w_down": _B_in["w_down"],
    }

def reference(A_x, A_k_cache, A_v_cache, A_wq, A_wo, B_x, B_w_r, B_w_gate, B_w_up, B_w_down):
    def _A_ref(x, k_cache, v_cache, wq, wo):
        B, Sq, D = x.shape
        H, Dh = 32, 192
        q = (lambda x, *d: x.transpose(*d))((x @ wq).reshape(B, Sq, H, Dh), 0, 2, 1, 3)
        scores = jnp.einsum("bhqd,bhkd->bhqk", q, k_cache) * (Dh ** -0.5)
        p = _softmax(scores, axis=-1)
        o = jnp.einsum("bhqk,bhkd->bhqd", p, v_cache)
        return (lambda x, *d: x.transpose(*d))(o, 0, 2, 1, 3).reshape(B, Sq, H * Dh) @ wo

    def _B_ref(x, w_r, w_gate, w_up, w_down):
        B, S, D = x.shape
        C = 1
        r = x @ w_r
        idx = jnp.argsort(-r, axis=-1)[:, :C]
        idx_e = jnp.repeat(idx.reshape(B, C, 1), D, axis=2)
        x_sel = jnp.take_along_axis(x, idx_e, axis=1)
        g = _silu(x_sel @ w_gate)
        u = x_sel @ w_up
        y = (g * u) @ w_down
        r_sel = _sigmoid(jnp.take_along_axis(r, idx, axis=1))
        y = y * r_sel.reshape(B, C, 1)
        b_off = (jnp.arange(B) * S).reshape(B, 1)
        flat_idx = (idx + b_off).reshape(B * C)
        zero = (x * 0.0).reshape(B * S, D)
        upd = _scatter_add(zero, flat_idx, y.reshape(B * C, D), axis=0)
        return x + upd.reshape(B, S, D)

    x = A_x
    h = x + _A_ref(_layernorm(x, axis=-1), A_k_cache, A_v_cache, A_wq, A_wo)
    h2 = h + _B_ref(_layernorm(h, axis=-1), B_w_r, B_w_gate, B_w_up, B_w_down)
    return h2
```

```python
import functools

import jax
import jax.numpy as jnp
import jax.experimental.pallas as pl
import jax.experimental.pallas.tpu as pltpu

_EPS = 1e-5
_NB = 3
_NS = 6
_CW = 1024
_LAG = 10
_FW = 256
OPT = dict(lag=_LAG, no=4, os=8, orow=24, wmode=0, fmode=0, vph=0, compute=True, nobc=False)


def _layernorm(x):
    m = jnp.mean(x, axis=-1, keepdims=True)
    d = x - m
    v = jnp.mean(d * d, axis=-1, keepdims=True)
    return d / jnp.sqrt(v + _EPS)


def _dot(a, b):
    return jnp.dot(a, b, preferred_element_type=jnp.float32)


def _dot_nt(a, b):
    return jax.lax.dot_general(
        a, b, (((1,), (1,)), ((), ())), preferred_element_type=jnp.float32
    )


def _wait_all(buf, sem):
    pltpu.make_async_copy(buf, buf, sem).wait()


def _loop(lo, hi, fn):
    jax.lax.fori_loop(lo, hi, lambda i, c: fn(i), None)


def _body(
    x_hbm, kt_hbm, vt_hbm, wq_hbm, wo_hbm, wr_hbm, wg_hbm, wu_hbm, wd_hbm,
    out_ref,
    kbuf, vbuf, wqbuf, wobuf, wgbuf, wubuf, wdbuf, xbuf, wrbuf,
    q_scr, o_scr, acc_scr, m_scr, l_scr,
    ksem, vsem, msem, gsem, usem, dsem, osem,
    *, B, H, Dh, Sk, D, F, opt,
):
    P = 2 * Dh
    n_pairs = H // 2
    G = Sk // _CW
    RT = P // _NS // 8
    assert RT == G
    n_steps = n_pairs * B * G
    NF = F // _FW
    LAG = opt["lag"]
    scale = Dh ** -0.5

    def issue_kv(t):
        s = t // G
        n = (s % B) * n_pairs + s // B
        r = t % G
        slot = s % _NB

        def half(c):
            cols = pl.ds(pl.multiple_of(c * _CW, _CW), _CW)
            vcols = pl.ds(pl.multiple_of(((c + opt["vph"]) % G) * _CW, _CW), _CW)
            for f in range(0, _NS, 2):
                two = pl.ds(f, 2)
                pltpu.make_async_copy(
                    kt_hbm.at[n, two, r, :, cols], kbuf.at[slot, two, r, :, cols], ksem.at[slot]
                ).start(priority=0)
                pltpu.make_async_copy(
                    vt_hbm.at[n, two, r, :, vcols], vbuf.at[slot, two, r, :, vcols], vsem.at[slot]
                ).start(priority=1)

        _loop(0, G, half)

    def issue_wq():
        if opt["wmode"] == 0:
            def piece(i):
                r = i // 3
                cols = pl.ds(pl.multiple_of((i % 3) * 2048, 2048), 2048)
                for f in range(5):
                    for q in range(2):
                        pltpu.make_async_copy(
                            wq_hbm.at[f + 5 * q, r, :, cols], wqbuf.at[f + 5 * q, r, :, cols], msem.at[2]
                        ).start(priority=q)

            _loop(0, 24, piece)
        else:
            prs = {1: [(0, 1), (2, 3), (4, 5), (6, 7), (8, 9)], 2: [(0, 4), (1, 5), (2, 6), (3, 7), (8, 9)]}[opt["wmode"]]
            def piece(i):
                r = i // 3
                for c in range(2):
                    cols = pl.ds(pl.multiple_of(((i % 3) * 2 + c) * 1024, 1024), 1024)
                    for f in range(5):
                        two = pl.ds(2 * f, 2)
                        pltpu.make_async_copy(
                            wq_hbm.at[two, r, :, cols], wqbuf.at[two, r, :, cols], msem.at[2]
                        ).start(priority=(f + c) % 2)

            _loop(0, 24, piece)

    NO = opt["no"]
    def issue_wo(j):
        ns, rows_per = opt["os"], opt["orow"]
        part = H * Dh // NO
        k = part // ns // rows_per
        assert k * ns * rows_per == part

        def piece(i):
            for f in range(ns):
                rows = pl.ds(pl.multiple_of(j * part + f * (part // ns) + i * rows_per, 8), rows_per)
                pltpu.make_async_copy(wo_hbm.at[rows, :], wobuf.at[rows, :], osem.at[j]).start(priority=f % 2)

        _loop(0, k, piece)

    def issue_gate_up(f):
        cols = pl.ds(pl.multiple_of(f * _FW, _FW), _FW)
        for r in range(0, D, 64):
            rows = pl.ds(r, 64)
            pltpu.make_async_copy(wg_hbm.at[rows, cols], wgbuf.at[f, rows, :], gsem.at[f]).start(priority=0)
            pltpu.make_async_copy(wu_hbm.at[rows, cols], wubuf.at[f, rows, :], usem.at[f]).start(priority=1)

    def issue_down(f):
        for i, r in enumerate(range(0, _FW, 32)):
            pltpu.make_async_copy(
                wd_hbm.at[pl.ds(pl.multiple_of(f * _FW + r, 32), 32), :],
                wdbuf.at[f, pl.ds(r, 32), :],
                dsem.at[f],
            ).start(priority=i % 2)

    x_cp = pltpu.make_async_copy(x_hbm, xbuf, msem.at[0])
    wr_cp = pltpu.make_async_copy(wr_hbm, wrbuf, msem.at[1])
    x_cp.start()
    wr_cp.start(priority=1)
    issue_wq()
    _loop(0, 2, issue_kv)

    x_cp.wait()
    x4 = xbuf[...].astype(jnp.float32)
    x = jnp.concatenate([x4, x4], axis=0)
    xn = _layernorm(x).astype(jnp.bfloat16)
    row = jax.lax.broadcasted_iota(jnp.int32, (2 * B, P), 0)
    col = jax.lax.broadcasted_iota(jnp.int32, (2 * B, P), 1)
    diag = (row < B) == (col < Dh)
    o_scr[...] = jnp.zeros_like(o_scr)

    _loop(2, LAG, issue_kv)
    _wait_all(wqbuf, msem.at[2])

    def step(t):
        s = t // G
        p = s // B
        b = s % B
        g = t % G
        slot = s % _NB
        pcols = pl.ds(pl.multiple_of(p * P, P), P)
        cols = pl.ds(pl.multiple_of(g * _CW, _CW), _CW)
        ahead = t + LAG - n_steps

        @pl.when(ahead < 0)
        def _():
            issue_kv(t + LAG)

        @pl.when(jnp.logical_and(ahead >= 0, ahead < NO))
        def _():
            issue_wo(ahead)

        @pl.when(jnp.logical_and(ahead >= NO, ahead < NO + NF // 2))
        def _():
            _loop(2 * (ahead - NO), 2 * (ahead - NO) + 2, issue_gate_up)

        @pl.when(t % (B * G) == 0)
        def _():
            q_scr[...] = jnp.where(diag, _dot(xn, wqbuf[:, :, :, pcols].reshape(D, P)), 0.0)

        @pl.when(g == 0)
        def _():
            m_scr[...] = jnp.full_like(m_scr, -jnp.inf)
            l_scr[...] = jnp.zeros_like(l_scr)
            acc_scr[...] = jnp.zeros_like(acc_scr)
            _wait_all(kbuf.at[slot], ksem.at[slot])
            _wait_all(vbuf.at[slot], vsem.at[slot])

        if opt["compute"]:
            k = kbuf[slot, :, :, :, cols].reshape(P, _CW)
            sc = _dot(q_scr[...].astype(jnp.bfloat16), k) * scale
            m_old = m_scr[...]
            m_new = jnp.maximum(m_old, jnp.max(sc, axis=-1, keepdims=True))
            m_sub = jnp.where(m_new == -jnp.inf, 0.0, m_new)
            e = jnp.exp(sc - m_sub)
            alpha = jnp.exp(m_old - m_sub)
            m_scr[...] = m_new
            l_scr[...] = alpha * l_scr[...] + jnp.sum(e, axis=-1, keepdims=True)
            v = vbuf[slot, :, :, :, cols].reshape(P, _CW)
            acc_scr[...] = alpha * acc_scr[...] + _dot_nt(e.astype(jnp.bfloat16), v)

        @pl.when(g == G - 1)
        def _():
            o = jnp.where(diag, acc_scr[...] / l_scr[...], 0.0)
            o_scr[p] = jnp.where(row % B == b, o, o_scr[p])

    assert LAG >= NO + NF // 2
    _loop(0, n_steps, step)

    attn = jnp.zeros((2 * B, D), jnp.float32)
    ppo = n_pairs // NO
    for j in range(NO):
        _loop(j * NF // NO, (j + 1) * NF // NO, issue_down)
        _wait_all(wobuf.at[pl.ds(j * ppo * P, ppo * P)], osem.at[j])
        for p in range(j * ppo, (j + 1) * ppo):
            attn = attn + _dot(o_scr[p].astype(jnp.bfloat16), wobuf[pl.ds(p * P, P), :])
    h = x + attn + pltpu.roll(attn, B, 0)
    hn = _layernorm(h)
    hb = hn.astype(jnp.bfloat16)
    wr_cp.wait()
    r = jnp.sum(hn * wrbuf[...].astype(jnp.float32).reshape(1, D), axis=-1, keepdims=True)
    acts = []
    for f in range(NF):
        _wait_all(wgbuf.at[f], gsem.at[f])
        _wait_all(wubuf.at[f], usem.at[f])
        gate = _dot(hb, wgbuf[f])
        up = _dot(hb, wubuf[f])
        acts.append((gate * jax.nn.sigmoid(gate) * up).astype(jnp.bfloat16))
    y = jnp.zeros((2 * B, D), jnp.float32)
    for f in range(NF):
        _wait_all(wdbuf.at[f], dsem.at[f])
        y = y + _dot(acts[f], wdbuf[f])
    y = y * jax.nn.sigmoid(r)
    out = h + (hn + (hn * 0.0 + y))
    out_ref[...] = out[:B].astype(out_ref.dtype)


def build(**kw):
    opt = dict(OPT, **kw)

    @jax.jit
    def fn(A_x, A_k_cache, A_v_cache, A_wq, A_wo, B_x, B_w_r, B_w_gate, B_w_up, B_w_down):
        del B_x
        B, Sq, D = A_x.shape
        _, H, Sk, Dh = A_k_cache.shape
        F = B_w_gate.shape[1]
        P = 2 * Dh
        dt = A_k_cache.dtype
        f32 = jnp.float32
        slab = (_NS, P // _NS // 8, 8, Sk)
        kt = jnp.swapaxes(A_k_cache, 2, 3).reshape(B * H // 2, *slab)
        vt = jnp.swapaxes(A_v_cache, 2, 3).reshape(B * H // 2, *slab)
        wq = A_wq.reshape(D // 64, 8, 8, H * Dh)
        out = pl.pallas_call(
            functools.partial(_body, B=B, H=H, Dh=Dh, Sk=Sk, D=D, F=F, opt=opt),
            in_specs=[pl.BlockSpec(memory_space=pl.ANY)] * 9,
            out_specs=pl.BlockSpec(memory_space=pltpu.VMEM),
            out_shape=jax.ShapeDtypeStruct((B, D), A_x.dtype),
            scratch_shapes=[
                pltpu.VMEM((_NB, *slab), dt),
                pltpu.VMEM((_NB, *slab), dt),
                pltpu.VMEM(wq.shape, dt),
                pltpu.VMEM(A_wo.shape, dt),
                pltpu.VMEM((F // _FW, D, _FW), dt),
                pltpu.VMEM((F // _FW, D, _FW), dt),
                pltpu.VMEM((F // _FW, _FW, D), dt),
                pltpu.VMEM((B, D), dt),
                pltpu.VMEM((D,), dt),
                pltpu.VMEM((2 * B, P), f32),
                pltpu.VMEM((H // 2, 2 * B, P), f32),
                pltpu.VMEM((2 * B, P), f32),
                pltpu.VMEM((2 * B, 1), f32),
                pltpu.VMEM((2 * B, 1), f32),
                pltpu.SemaphoreType.DMA((_NB,)),
                pltpu.SemaphoreType.DMA((_NB,)),
                pltpu.SemaphoreType.DMA((4,)),
                pltpu.SemaphoreType.DMA((F // _FW,)),
                pltpu.SemaphoreType.DMA((F // _FW,)),
                pltpu.SemaphoreType.DMA((F // _FW,)),
                pltpu.SemaphoreType.DMA((opt["no"],)),
            ],
            compiler_params=pltpu.CompilerParams(
                vmem_limit_bytes=90 * 1024 * 1024, disable_bounds_checks=opt["nobc"]
            ),
        )(A_x.reshape(B, D), kt, vt, wq, A_wo, B_w_r, B_w_gate, B_w_up, B_w_down)
        return out.reshape(B, Sq, D)

    return fn


_kernel = build(lag=9)


def pallas_sequential_preLN__mha_block_cached__moe_arch_mod__decode_kernel(
    A_x, A_k_cache, A_v_cache, A_wq, A_wo, B_x, B_w_r, B_w_gate, B_w_up, B_w_down
):
    return _kernel(
        A_x, A_k_cache, A_v_cache, A_wq, A_wo, B_x, B_w_r, B_w_gate, B_w_up, B_w_down
    )
```

```python
import functools

import jax
import jax.numpy as jnp
import jax.experimental.pallas as pl
import jax.experimental.pallas.tpu as pltpu

_EPS = 1e-5
_NB = 3
_NS = 6
_CW = 1024
_LAG = 9
OPT = dict(no=6, os=8, orow=32, gr=32, gw=512, dr=16, ds=4, nobc=False, nosc=False, compute=True,
           dp=(512,) * 3, dat=(0, 4, 8), flags=None, wq=0)


def _layernorm(x):
    m = jnp.mean(x, axis=-1, keepdims=True)
    d = x - m
    v = jnp.mean(d * d, axis=-1, keepdims=True)
    return d / jnp.sqrt(v + _EPS)


def _dot(a, b):
    return jnp.dot(a, b, preferred_element_type=jnp.float32)


def _dot_nt(a, b):
    return jax.lax.dot_general(
        a, b, (((1,), (1,)), ((), ())), preferred_element_type=jnp.float32
    )


def _wait_for(sem, *bufs):
    for buf in bufs:
        pltpu.make_async_copy(buf, buf, sem).wait()


def _loop(lo, hi, fn):
    jax.lax.fori_loop(lo, hi, lambda i, carry: fn(i), None)


def _divmod(i, n):
    if n & (n - 1) == 0:
        return jax.lax.shift_right_logical(i, n.bit_length() - 1), i & (n - 1)
    return jax.lax.div(i, n), jax.lax.rem(i, n)


def _block(i, n):
    return pl.ds(pl.multiple_of(i * n, n), n)


def _body(
    x_hbm, kt_hbm, vt_hbm, wq_hbm, wo_hbm, wr_hbm, wg_hbm, wu_hbm, wd_hbm,
    out_ref,
    kbuf, vbuf, wqbuf, wobuf, wgbuf, wubuf, wdbuf, xbuf, wrbuf,
    q_scr, o_scr, acc_scr, m_scr, l_scr, sem,
    *, B, H, Dh, Sk, D, F, opt,
):
    P = 2 * Dh
    n_pairs = H // 2
    G = Sk // _CW
    n_slabs = n_pairs * B
    n_steps = n_slabs * G
    NO = opt["no"]
    NF = _LAG - NO
    FW = F // NF
    scale = Dh ** -0.5

    def issue_kv(t):
        s, r = _divmod(t, G)
        p, b = _divmod(s, B)
        slot = _divmod(s, _NB)[1]

        def run(c):
            for f in range(0, _NS, 2):
                at = (pl.ds(f, 2), r, slice(None), _block(c, _CW))
                for q, (hbm, buf) in enumerate(((kt_hbm, kbuf), (vt_hbm, vbuf))):
                    pltpu.make_async_copy(
                        hbm.at[(b * n_pairs + p, *at)], buf.at[(slot, *at)], sem.at[slot]
                    ).start(priority=q)

        _loop(0, G, run)

    def issue_wq(i):
        r, c = _divmod(i, 3)
        if opt["wq"] == 0:
            for f in range(5):
                for q in range(2):
                    at = (f + 5 * q, r, slice(None), _block(c, 2048))
                    pltpu.make_async_copy(wq_hbm.at[at], wqbuf.at[at], sem.at[_NB - 1]).start(priority=q)
        else:
            for h in range(2):
                for f in range(5):
                    at = (pl.ds(2 * f, 2), r, slice(None), _block(2 * c + h, 1024))
                    pltpu.make_async_copy(wq_hbm.at[at], wqbuf.at[at], sem.at[_NB - 1]).start(priority=(f + h) % 2)

    o_part = H * Dh // NO
    o_units = o_part // opt["os"] // opt["orow"]
    assert o_units * opt["os"] * opt["orow"] == o_part

    def issue_wo(j, s):
        def piece(i):
            for f in range(opt["os"]):
                rows = _block((f * NO + j) * o_units + i, opt["orow"])
                pltpu.make_async_copy(wo_hbm.at[rows, :], wobuf.at[rows, :], s).start(priority=f % 2)

        _loop(0, o_units, piece)

    def issue_gate_up(f, s):
        def piece(i):
            for a in range(4):
                for c in range(FW // opt["gw"]):
                    rows = _block(a * (D // 4 // opt["gr"]) + i, opt["gr"])
                    for q, (hbm, buf) in enumerate(((wg_hbm, wgbuf), (wu_hbm, wubuf))):
                        pltpu.make_async_copy(
                            hbm.at[rows, _block(f * (FW // opt["gw"]) + c, opt["gw"])],
                            buf.at[f, rows, pl.ds(c * opt["gw"], opt["gw"])], s
                        ).start(priority=q)

        _loop(0, D // 4 // opt["gr"], piece)

    def issue_down(r0, n, s):
        k = n // opt["ds"] // opt["dr"]

        def piece(i):
            for f in range(opt["ds"]):
                rows = pl.ds(pl.multiple_of(r0 + (f * k + i) * opt["dr"], opt["dr"]), opt["dr"])
                pltpu.make_async_copy(wd_hbm.at[rows, :], wdbuf.at[rows, :], s).start(priority=f % 2)

        _loop(0, k, piece)

    def tail_sem(i):
        return sem.at[_divmod(n_slabs + i, _NB)[1]]

    pltpu.make_async_copy(x_hbm, xbuf, sem.at[_NB - 1]).start()
    pltpu.make_async_copy(wr_hbm, wrbuf, sem.at[_NB - 1]).start(priority=1)
    _loop(0, 24, issue_wq)
    _loop(0, _LAG, issue_kv)
    _wait_for(sem.at[_NB - 1], xbuf, wrbuf, wqbuf)

    x4 = xbuf[...].astype(jnp.float32)
    x = jnp.concatenate([x4, x4], axis=0)
    xn = _layernorm(x).astype(jnp.bfloat16)
    row = jax.lax.broadcasted_iota(jnp.int32, (2 * B, P), 0)
    col = jax.lax.broadcasted_iota(jnp.int32, (2 * B, P), 1)
    diag = (row < B) == (col < Dh)
    o_scr[...] = jnp.zeros_like(o_scr)

    def step(t):
        s, g = _divmod(t, G)
        p, b = _divmod(s, B)
        slot = _divmod(s, _NB)[1]
        ahead = t + _LAG - n_steps

        @pl.when(ahead < 0)
        def _():
            issue_kv(t + _LAG)

        @pl.when(ahead >= 0)
        def _():
            @pl.when(ahead >= _NB)
            def _():
                _wait_for(tail_sem(ahead), wobuf.at[pl.ds(0, o_part)])

            @pl.when(ahead < NO)
            def _():
                issue_wo(ahead, tail_sem(ahead))

            @pl.when(ahead >= NO)
            def _():
                issue_gate_up(ahead - NO, tail_sem(ahead))

        @pl.when(g == 0)
        def _():
            @pl.when(b == 0)
            def _():
                q = _dot(xn, wqbuf[:, :, :, _block(p, P)].reshape(D, P))
                q_scr[...] = jnp.where(diag, q, 0.0)

            m_scr[...] = jnp.full_like(m_scr, -jnp.inf)
            l_scr[...] = jnp.zeros_like(l_scr)
            acc_scr[...] = jnp.zeros_like(acc_scr)
            _wait_for(sem.at[slot], kbuf.at[slot], vbuf.at[slot])

        if opt["compute"]:
            k = kbuf[slot, :, :, :, _block(g, _CW)].reshape(P, _CW)
            sc = _dot(q_scr[...].astype(jnp.bfloat16), k) * scale
            m_old = m_scr[...]
            m_new = jnp.maximum(m_old, jnp.max(sc, axis=-1, keepdims=True))
            m_sub = jnp.where(m_new == -jnp.inf, 0.0, m_new)
            e = jnp.exp(sc - m_sub)
            alpha = jnp.exp(m_old - m_sub)
            m_scr[...] = m_new
            l_scr[...] = alpha * l_scr[...] + jnp.sum(e, axis=-1, keepdims=True)
            v = vbuf[slot, :, :, :, _block(g, _CW)].reshape(P, _CW)
            acc_scr[...] = alpha * acc_scr[...] + _dot_nt(e.astype(jnp.bfloat16), v)

        @pl.when(g == G - 1)
        def _():
            o = jnp.where(diag, acc_scr[...] / l_scr[...], 0.0)
            o_scr[p] = jnp.where(row % B == b, o, o_scr[p])

    assert NO == _LAG - _NB
    _loop(0, n_steps, step)

    dp = opt["dp"]
    dsem = [sem.at[_NB + i] for i in range(len(dp))]
    attn = jnp.zeros((2 * B, D), jnp.float32)
    for p in range(n_pairs):
        for i, at in enumerate(opt["dat"]):
            if at == p:
                issue_down(sum(dp[:i]), dp[i], dsem[i])
        attn = attn + _dot(o_scr[p].astype(jnp.bfloat16), wobuf[pl.ds(p * P, P), :])
    h = x + attn + pltpu.roll(attn, B, 0)
    hn = _layernorm(h)
    hb = hn.astype(jnp.bfloat16)
    r = jnp.sum(hn * wrbuf[...].astype(jnp.float32).reshape(1, D), axis=-1, keepdims=True)
    r_gate = jax.nn.sigmoid(r)
    acts = []
    for f in range(NF):
        _wait_for(sem.at[(n_slabs + NO + f) % _NB], wgbuf.at[f], wubuf.at[f])
        gate = _dot(hb, wgbuf[f])
        acts.append((gate * jax.nn.sigmoid(gate) * _dot(hb, wubuf[f])).astype(jnp.bfloat16))
    act = jnp.concatenate(acts, axis=1)
    y = jnp.zeros((2 * B, D), jnp.float32)
    for i, n in enumerate(dp):
        r0 = sum(dp[:i])
        _wait_for(dsem[i], wdbuf.at[pl.ds(r0, n)])
        y = y + _dot(act[:, r0:r0 + n], wdbuf[pl.ds(r0, n), :])
    out = h + (hn + (hn * 0.0 + y * r_gate))
    out_ref[...] = out[:B].astype(out_ref.dtype)


def build(**kw):
    opt = dict(OPT, **kw)

    @jax.jit
    def fn(A_x, A_k_cache, A_v_cache, A_wq, A_wo, B_x, B_w_r, B_w_gate, B_w_up, B_w_down):
        del B_x
        B, Sq, D = A_x.shape
        _, H, Sk, Dh = A_k_cache.shape
        F = B_w_gate.shape[1]
        P = 2 * Dh
        NF = _LAG - opt["no"]
        dt = A_k_cache.dtype
        f32 = jnp.float32
        slab = (_NS, P // _NS // 8, 8, Sk)
        kt = jnp.swapaxes(A_k_cache, 2, 3).reshape(B * H // 2, *slab)
        vt = jnp.swapaxes(A_v_cache, 2, 3).reshape(B * H // 2, *slab)
        wq = A_wq.reshape(D // 64, 8, 8, H * Dh)
        out = pl.pallas_call(
            functools.partial(_body, B=B, H=H, Dh=Dh, Sk=Sk, D=D, F=F, opt=opt),
            in_specs=[pl.BlockSpec(memory_space=pl.ANY)] * 9,
            out_specs=pl.BlockSpec(memory_space=pltpu.VMEM),
            out_shape=jax.ShapeDtypeStruct((B, D), A_x.dtype),
            scratch_shapes=[
                pltpu.VMEM((_NB, *slab), dt),
                pltpu.VMEM((_NB, *slab), dt),
                pltpu.VMEM(wq.shape, dt),
                pltpu.VMEM(A_wo.shape, dt),
                pltpu.VMEM((NF, D, F // NF), dt),
                pltpu.VMEM((NF, D, F // NF), dt),
                pltpu.VMEM((F, D), dt),
                pltpu.VMEM((B, D), dt),
                pltpu.VMEM((D,), dt),
                pltpu.VMEM((2 * B, P), f32),
                pltpu.VMEM((H // 2, 2 * B, P), f32),
                pltpu.VMEM((2 * B, P), f32),
                pltpu.VMEM((2 * B, 1), f32),
                pltpu.VMEM((2 * B, 1), f32),
                pltpu.SemaphoreType.DMA((_NB + len(opt["dp"]),)),
            ],
            compiler_params=pltpu.CompilerParams(
                vmem_limit_bytes=90 * 1024 * 1024, disable_bounds_checks=opt["nobc"], flags=opt["flags"],
                disable_semaphore_checks=opt["nosc"],
            ),
        )(A_x.reshape(B, D), kt, vt, wq, A_wo, B_w_r, B_w_gate, B_w_up, B_w_down)
        return out.reshape(B, Sq, D)

    return fn


_kernel = build(dat=(2, 7, 12))


def pallas_sequential_preLN__mha_block_cached__moe_arch_mod__decode_kernel(
    A_x, A_k_cache, A_v_cache, A_wq, A_wo, B_x, B_w_r, B_w_gate, B_w_up, B_w_down
):
    return _kernel(
        A_x, A_k_cache, A_v_cache, A_wq, A_wo, B_x, B_w_r, B_w_gate, B_w_up, B_w_down
    )
```

```python
import functools

import jax
import jax.numpy as jnp
import jax.experimental.pallas as pl
import jax.experimental.pallas.tpu as pltpu

_EPS = 1e-5
_NB = 3
_NH = 4
_SR = 64
_CW = 1024
_LAG = 9
OPT = dict(no=6, os=8, orow=32, gr=32, gw=512, dr=16, ds=4, nobc=False, nosc=False, compute=True,
           dp=(512,) * 3, dat=(1, 3, 6), flags=None, wq=0, lead=26, ps=1, pe=1, s2=0, sub=1)


def _layernorm(x):
    m = jnp.mean(x, axis=-1, keepdims=True)
    d = x - m
    v = jnp.mean(d * d, axis=-1, keepdims=True)
    return d / jnp.sqrt(v + _EPS)


def _dot(a, b):
    return jnp.dot(a, b, preferred_element_type=jnp.float32)


def _dot_nt(a, b):
    return jax.lax.dot_general(
        a, b, (((1,), (1,)), ((), ())), preferred_element_type=jnp.float32
    )


def _wait_for(sem, *bufs):
    for buf in bufs:
        pltpu.make_async_copy(buf, buf, sem).wait()


def _loop(lo, hi, fn):
    jax.lax.fori_loop(lo, hi, lambda i, carry: fn(i), None)


def _divmod(i, n):
    if n & (n - 1) == 0:
        return jax.lax.shift_right_logical(i, n.bit_length() - 1), i & (n - 1)
    return jax.lax.div(i, n), jax.lax.rem(i, n)


def _block(i, n):
    return pl.ds(i * n if isinstance(i, int) else pl.multiple_of(i * n, n), n)


def _body(
    x_hbm, kt_hbm, vt_hbm, wq_hbm, wo_hbm, wr_hbm, wg_hbm, wu_hbm, wd_hbm,
    out_ref,
    ring, wqbuf, wobuf, wgbuf, wubuf, wdbuf, xbuf, wrbuf,
    q_scr, s_scr, o_scr, acc_scr, m_scr, l_scr, sem,
    *, B, H, Dh, Sk, D, F, opt,
):
    P = _NH * Dh
    NS = P // _SR
    n_quads = H // _NH
    G = Sk // _CW
    n_slabs = 2 * n_quads * B
    n_steps = n_slabs * G
    n_units = n_steps * G
    NO = opt["no"]
    NF = _LAG - NO
    FW = F // NF
    scale = Dh ** -0.5
    pieces = NS // 4
    lead_units, lead_pieces = divmod(opt["lead"], pieces)

    def rows_of(t):
        s, r = _divmod(t, G)
        j, b = _divmod(_divmod(s, 2)[0], B)
        return b * n_quads + j, _divmod(s, _NB)[1], r, s

    def start_piece(hbm, rows, c, f, queue):
        n, slot, r, _ = rows
        at = (f, slice(None), queue) if opt["s2"] else (f, queue, slice(None))
        at = (*at, r, slice(None), _block(c, _CW))
        pltpu.make_async_copy(hbm.at[(n, *at)], ring.at[(slot, *at)], sem.at[slot]).start(priority=queue)

    def with_cache(rows, fn):
        s = rows[-1]
        for i, hbm in enumerate((kt_hbm, vt_hbm)):
            pl.when(jnp.logical_and(s & 1 == i, s < n_slabs))(functools.partial(fn, hbm))

    assert lead_units == G or opt['lead'] == G * pieces + 3 or opt["lead"] == G * pieces - 1
    skew = opt["lead"] - G * pieces

    def start_down0(c, f):
        r0 = c * 64 + f * 24
        rows = pl.ds(r0 if isinstance(r0, int) else pl.multiple_of(r0, 8), 24 if f < 2 else 16)
        pltpu.make_async_copy(wd_hbm.at[rows, :], wdbuf.at[rows, :], sem.at[_NB]).start(priority=1)

    def issue_kv(t):
        first, second, third = rows_of(t), rows_of(t + 1), rows_of(t + 2)

        def body(hbm0, hbm1):
            def column(c):
                for f in range(pieces):
                    start_piece(hbm0, first, c, f, 0)
                    if hbm1 is not None:
                        carry, f1 = divmod(f + skew, pieces)
                        start_piece(hbm1, second, c + carry, f1, 1)
                    elif opt["pe"]:
                        start_down0(c, f)

            _loop(0, G - 1, column)
            for f in range(pieces):
                start_piece(hbm0, first, G - 1, f, 0)
                if f + skew >= pieces:
                    with_cache(third, lambda hbm: start_piece(hbm, third, 0, f + skew - pieces, 1))
                elif hbm1 is not None:
                    start_piece(hbm1, second, G - 1, f + skew, 1)
                if hbm1 is None and opt["pe"]:
                    start_down0(G - 1, f)

        @pl.when(t + 1 < n_steps)
        def _():
            with_cache(first, lambda hbm0: with_cache(second, functools.partial(body, hbm0)))

        @pl.when(t + 1 == n_steps)
        def _():
            body(vt_hbm, None)

    def start_wq(f, r, c, queue):
        at = (f, r, slice(None), _block(c, 2048))
        pltpu.make_async_copy(wq_hbm.at[at], wqbuf.at[at], sem.at[_NB - 1]).start(priority=queue)

    def issue_wq(r):
        n = 9 if opt["ps"] else 10
        for h in range(2):
            for c in range(3):
                for f in range(n):
                    start_wq(f, 2 * r + h, c, ((h * 3 + c) * n + f) % 2)

    o_part = H * Dh // NO
    o_units = o_part // opt["os"] // opt["orow"]
    assert o_units * opt["os"] * opt["orow"] == o_part

    def issue_wo(j, s):
        def piece(i):
            for f in range(opt["os"]):
                rows = _block((f * NO + j) * o_units + i, opt["orow"])
                pltpu.make_async_copy(wo_hbm.at[rows, :], wobuf.at[rows, :], s).start(priority=f % 2)

        _loop(0, o_units, piece)

    def issue_gate_up(f, s):
        def piece(i):
            for a in range(4):
                for c in range(FW // opt["gw"]):
                    rows = _block(a * (D // 4 // opt["gr"]) + i, opt["gr"])
                    for q, (hbm, buf) in enumerate(((wg_hbm, wgbuf), (wu_hbm, wubuf))):
                        pltpu.make_async_copy(
                            hbm.at[rows, _block(f * (FW // opt["gw"]) + c, opt["gw"])],
                            buf.at[f, rows, pl.ds(c * opt["gw"], opt["gw"])], s
                        ).start(priority=q)

        _loop(0, D // 4 // opt["gr"], piece)

    def issue_down(r0, n, s):
        k = n // opt["ds"] // opt["dr"]

        def piece(i):
            for f in range(opt["ds"]):
                rows = pl.ds(pl.multiple_of(r0 + (f * k + i) * opt["dr"], opt["dr"]), opt["dr"])
                pltpu.make_async_copy(wd_hbm.at[rows, :], wdbuf.at[rows, :], s).start(priority=f % 2)

        _loop(0, k, piece)

    def tail_sem(i):
        return sem.at[_divmod(n_slabs + i, _NB)[1]]

    pltpu.make_async_copy(x_hbm, xbuf, sem.at[_NB - 1]).start()
    pltpu.make_async_copy(wr_hbm, wrbuf, sem.at[_NB - 1]).start(priority=1)
    _loop(0, 4, issue_wq)

    def head_start(c):
        for f in range(pieces):
            if opt["ps"]:
                start_wq(9, c, f, 0)
            start_piece(kt_hbm, (0, 0, 0, 0), c, f, 1)

    _loop(0, G, head_start)
    for f in range(skew):
        start_piece(kt_hbm, (0, 0, 1, 0), 0, f, 1)
    _loop(0, _LAG, issue_kv)
    _wait_for(sem.at[_NB - 1], xbuf, wrbuf, wqbuf)

    x4 = xbuf[...].astype(jnp.float32)
    x = jnp.concatenate([x4, x4], axis=0)
    xn = _layernorm(x).astype(jnp.bfloat16)
    row = jax.lax.broadcasted_iota(jnp.int32, (8, P), 0)
    col = jax.lax.broadcasted_iota(jnp.int32, (8, P), 1)
    head_row = row & (_NH - 1)
    diag = jnp.logical_and(col >= head_row * Dh, col < (head_row + 1) * Dh)
    o_scr[...] = jnp.zeros_like(o_scr)

    def step(t):
        s, g = _divmod(t, G)
        j, b = _divmod(_divmod(s, 2)[0], B)
        slot = _divmod(s, _NB)[1]
        ahead = t + _LAG - n_steps

        @pl.when(ahead < 0)
        def _():
            issue_kv(t + _LAG)

        @pl.when(ahead >= 0)
        def _():
            @pl.when(ahead >= _NB)
            def _():
                _wait_for(tail_sem(ahead), wobuf.at[pl.ds(0, o_part)])

            @pl.when(ahead < NO)
            def _():
                issue_wo(ahead, tail_sem(ahead))

            @pl.when(ahead >= NO)
            def _():
                issue_gate_up(ahead - NO, tail_sem(ahead))

        @pl.when(g == 0)
        def _():
            _wait_for(sem.at[slot], ring.at[slot])

        def part():
            return ring[slot, :, :, :, :, :, _block(g, _CW)].reshape(P, _CW)

        @pl.when(s & 1 == 0)
        def _():
            @pl.when(g == 0)
            def _():
                q = _dot(xn, wqbuf[:, :, :, _block(j, P)].reshape(D, P))
                q = jnp.sum(jnp.where(row == b, q, 0.0), axis=0, keepdims=True)
                q_scr[...] = jnp.where(diag, q, 0.0)
                m_scr[...] = jnp.full_like(m_scr, -jnp.inf)

            if opt["compute"]:
                sc = _dot(q_scr[...].astype(jnp.bfloat16), part()) * scale
                s_scr[:, _block(g, _CW)] = sc
                m_scr[...] = jnp.maximum(m_scr[...], jnp.max(sc, axis=-1, keepdims=True))

        @pl.when(s & 1 == 1)
        def _():
            @pl.when(g == 0)
            def _():
                l_scr[...] = jnp.zeros_like(l_scr)
                acc_scr[...] = jnp.zeros_like(acc_scr)

            if opt["compute"]:
                e = jnp.exp(s_scr[:, _block(g, _CW)] - m_scr[...])
                l_scr[...] += jnp.sum(e, axis=-1, keepdims=True)
                acc_scr[...] += _dot_nt(e.astype(jnp.bfloat16), part())

            @pl.when(g == G - 1)
            def _():
                o = jnp.where(jnp.logical_and(diag, row < _NH), acc_scr[...] / l_scr[...], 0.0)
                o = jnp.sum(o, axis=0, keepdims=True)
                o_scr[j] = jnp.where(row == b, o, o_scr[j])

    assert NO == _LAG - _NB
    _loop(0, n_steps, step)

    dp = opt["dp"]
    dsem = [sem.at[_NB + i] for i in range(len(dp))]
    attn = jnp.zeros((8, D), jnp.float32)
    for p in range(n_quads):
        for i, at in enumerate(opt["dat"]):
            if at == p and (i or not opt['pe']):
                issue_down(sum(dp[:i]), dp[i], dsem[i])
        attn = attn + _dot(o_scr[p].astype(jnp.bfloat16), wobuf[pl.ds(p * P, P), :])
    h = x + attn
    hn = _layernorm(h)
    hb = hn.astype(jnp.bfloat16)
    r = jnp.sum(hn * wrbuf[...].astype(jnp.float32).reshape(1, D), axis=-1, keepdims=True)
    r_gate = jax.nn.sigmoid(r)
    acts = []
    for f in range(NF):
        _wait_for(sem.at[(n_slabs + NO + f) % _NB], wgbuf.at[f], wubuf.at[f])
        gate = _dot(hb, wgbuf[f])
        acts.append((gate * jax.nn.sigmoid(gate) * _dot(hb, wubuf[f])).astype(jnp.bfloat16))
    act = jnp.concatenate(acts, axis=1)
    y = jnp.zeros((2 * B, D), jnp.float32)
    for i, n in enumerate(dp):
        r0 = sum(dp[:i])
        _wait_for(dsem[i], wdbuf.at[pl.ds(r0, n)])
        y = y + _dot(act[:, r0:r0 + n], wdbuf[pl.ds(r0, n), :])
    out = h + (hn + (hn * 0.0 + y * r_gate))
    out_ref[...] = out[:B].astype(out_ref.dtype)


def build(**kw):
    opt = dict(OPT, **kw)

    @jax.jit
    def fn(A_x, A_k_cache, A_v_cache, A_wq, A_wo, B_x, B_w_r, B_w_gate, B_w_up, B_w_down):
        del B_x
        B, Sq, D = A_x.shape
        _, H, Sk, Dh = A_k_cache.shape
        F = B_w_gate.shape[1]
        P = _NH * Dh
        NF = _LAG - opt["no"]
        dt = A_k_cache.dtype
        f32 = jnp.float32
        slab = (P // _SR // 4, 2, 2, _SR // 8, 8, Sk)
        kt = jnp.swapaxes(A_k_cache, 2, 3).reshape(B * H // _NH, *slab)
        vt = jnp.swapaxes(A_v_cache, 2, 3).reshape(B * H // _NH, *slab)
        wq = A_wq.reshape(D // 64, 8, 8, H * Dh)
        out = pl.pallas_call(
            functools.partial(_body, B=B, H=H, Dh=Dh, Sk=Sk, D=D, F=F, opt=opt),
            in_specs=[pl.BlockSpec(memory_space=pl.ANY)] * 9,
            out_specs=pl.BlockSpec(memory_space=pltpu.VMEM),
            out_shape=jax.ShapeDtypeStruct((B, D), A_x.dtype),
            scratch_shapes=[
                pltpu.VMEM((_NB, *slab), dt),
                pltpu.VMEM(wq.shape, dt),
                pltpu.VMEM(A_wo.shape, dt),
                pltpu.VMEM((NF, D, F // NF), dt),
                pltpu.VMEM((NF, D, F // NF), dt),
                pltpu.VMEM((F, D), dt),
                pltpu.VMEM((B, D), dt),
                pltpu.VMEM((D,), dt),
                pltpu.VMEM((2 * B, P), f32),
                pltpu.VMEM((8, Sk), f32),
                pltpu.VMEM((H // _NH, 8, P), f32),
                pltpu.VMEM((2 * B, P), f32),
                pltpu.VMEM((2 * B, 1), f32),
                pltpu.VMEM((2 * B, 1), f32),
                pltpu.SemaphoreType.DMA((_NB + len(opt["dp"]),)),
            ],
            compiler_params=pltpu.CompilerParams(
                vmem_limit_bytes=90 * 1024 * 1024, disable_bounds_checks=opt["nobc"], flags=opt["flags"],
                disable_semaphore_checks=opt["nosc"],
            ),
        )(A_x.reshape(B, D), kt, vt, wq, A_wo, B_w_r, B_w_gate, B_w_up, B_w_down)
        return out.reshape(B, Sq, D)

    return fn


_kernel = build(s2=1)


def pallas_sequential_preLN__mha_block_cached__moe_arch_mod__decode_kernel(
    A_x, A_k_cache, A_v_cache, A_wq, A_wo, B_x, B_w_r, B_w_gate, B_w_up, B_w_down
):
    return _kernel(
        A_x, A_k_cache, A_v_cache, A_wq, A_wo, B_x, B_w_r, B_w_gate, B_w_up, B_w_down
    )
```

```python
import functools

import jax
import jax.numpy as jnp
import jax.experimental.pallas as pl
import jax.experimental.pallas.tpu as pltpu

_EPS = 1e-5
_ROWS = 8
_NH = 4
_SR = 64
_CW = 1024
_NB = 3
_LAG = 9
_SKEW = 2
_OW = 128
_FW = 512


def _layernorm(x):
    m = jnp.mean(x, axis=-1, keepdims=True)
    d = x - m
    v = jnp.mean(d * d, axis=-1, keepdims=True)
    return d / jnp.sqrt(v + _EPS)


def _dot(a, b):
    return jnp.dot(a, b, preferred_element_type=jnp.float32)


def _dot_nt(a, b):
    return jax.lax.dot_general(
        a, b, (((1,), (1,)), ((), ())), preferred_element_type=jnp.float32
    )


def _wait_for(sem, *bufs):
    for buf in bufs:
        pltpu.make_async_copy(buf, buf, sem).wait()


def _loop(n, fn):
    jax.lax.fori_loop(0, n, lambda i, carry: fn(i), None)


def _divmod(i, n):
    if n & (n - 1) == 0:
        return jax.lax.shift_right_logical(i, n.bit_length() - 1), i & (n - 1)
    return jax.lax.div(i, n), jax.lax.rem(i, n)


def _span(start, size, align):
    return pl.ds(start if isinstance(start, int) else pl.multiple_of(start, align), size)


def _block(i, size):
    return _span(i * size, size, size)


def _body(
    x_hbm, kt_hbm, vt_hbm, wq_hbm, wo_hbm, wr_hbm, wg_hbm, wu_hbm, wd_hbm,
    out_ref,
    ring, wqbuf, wobuf, wgbuf, wubuf, wdbuf, xbuf, wrbuf,
    q_scr, s_scr, m_scr, l_scr, acc_scr, o_scr, attn_scr, sem,
    *, B, H, Dh, Sk, D, F,
):
    P = _NH * Dh
    n_groups = H // _NH
    G = Sk // _CW
    pairs = P // _SR // 4
    n_slabs = 2 * n_groups * B
    n_steps = n_slabs * G
    NO = P // _OW
    NF = F // _FW
    scale = Dh ** -0.5

    def row_tile(t):
        s, r = _divmod(t, G)
        j, b = _divmod(_divmod(s, 2)[0], B)
        return b * n_groups + j, _divmod(s, _NB)[1], r, s

    def start_runs(hbm, tile, c, f, queue):
        n, slot, r, _ = tile
        at = (f, slice(None), queue, r, slice(None), _block(c, _CW))
        pltpu.make_async_copy(
            hbm.at[(n, *at)], ring.at[(slot, *at)], sem.at[slot]
        ).start(priority=queue)

    def with_cache(tile, fn):
        s = tile[-1]
        for i, hbm in enumerate((kt_hbm, vt_hbm)):
            pl.when(jnp.logical_and((s & 1) == i, s < n_slabs))(functools.partial(fn, hbm))

    def issue_cache(t):
        first, second, third = row_tile(t), row_tile(t + 1), row_tile(t + 2)

        def both(hbm0, hbm1):
            def column(c):
                for f in range(pairs):
                    start_runs(hbm0, first, c, f, 0)
                    carry, f1 = divmod(f + _SKEW, pairs)
                    start_runs(hbm1, second, c + carry, f1, 1)

            _loop(G - 1, column)
            for f in range(pairs):
                start_runs(hbm0, first, G - 1, f, 0)
                carry, f1 = divmod(f + _SKEW, pairs)
                if carry:
                    with_cache(third, lambda hbm: start_runs(hbm, third, 0, f1, 1))
                else:
                    start_runs(hbm1, second, G - 1, f1, 1)

        @pl.when(t + 1 < n_steps)
        def _():
            with_cache(first, lambda hbm0: with_cache(second, functools.partial(both, hbm0)))

        @pl.when(t + 1 == n_steps)
        def _():
            def column(c):
                for f, (r0, size) in enumerate(((0, 24), (24, 24), (48, 16))):
                    start_runs(vt_hbm, first, c, f, 0)
                    rows = _span(c * (_FW // G) + r0, size, _ROWS)
                    pltpu.make_async_copy(
                        wd_hbm.at[rows, :], wdbuf.at[0, rows, :], sem.at[_NB]
                    ).start(priority=1)

            _loop(G, column)

    def start_wq(f, r, c, queue):
        at = (f, r, slice(None), _block(c, H * Dh // pairs))
        pltpu.make_async_copy(wq_hbm.at[at], wqbuf.at[at], sem.at[_NB - 1]).start(priority=queue)

    def issue_wq(i):
        n = D // _SR - 1
        for h in range(2):
            for c in range(pairs):
                for f in range(n):
                    start_wq(f, 2 * i + h, c, ((h * pairs + c) * n + f) % 2)

    def head_start(c):
        for f in range(pairs):
            start_wq(D // _SR - 1, c, f, 0)
            start_runs(kt_hbm, (0, 0, 0, 0), c, f, 1)

    def issue_wo(part, s):
        def piece(i):
            for j in range(n_groups):
                pltpu.make_async_copy(
                    wo_hbm.at[_span(j * P + part * _OW + i * 32, 32, 32), :],
                    wobuf.at[part, j, _block(i, 32), :],
                    s,
                ).start(priority=j % 2)

        _loop(_OW // 32, piece)

    def issue_gate_up(f, s):
        def piece(i):
            for r0 in range(0, D, D // 4):
                rows = _span(r0 + i * 32, 32, 32)
                for queue, (hbm, buf) in enumerate(((wg_hbm, wgbuf), (wu_hbm, wubuf))):
                    pltpu.make_async_copy(
                        hbm.at[rows, _block(f, _FW)], buf.at[f, rows, :], s
                    ).start(priority=queue)

        _loop(D // 4 // 32, piece)

    def issue_down(f):
        def piece(i):
            for a, r0 in enumerate(range(0, _FW, _FW // 4)):
                pltpu.make_async_copy(
                    wd_hbm.at[_span(f * _FW + r0 + i * 16, 16, 16), :],
                    wdbuf.at[f, _span(r0 + i * 16, 16, 16), :],
                    sem.at[_NB + f],
                ).start(priority=a % 2)

        _loop(_FW // 4 // 16, piece)

    pltpu.make_async_copy(x_hbm, xbuf, sem.at[_NB - 1]).start()
    pltpu.make_async_copy(wr_hbm, wrbuf, sem.at[_NB - 1]).start(priority=1)
    _loop(_SR // _ROWS // 2, issue_wq)
    _loop(G, head_start)
    for f in range(_SKEW):
        start_runs(kt_hbm, (0, 0, 1, 0), 0, f, 1)
    _loop(_LAG, issue_cache)
    _wait_for(sem.at[_NB - 1], xbuf, wrbuf, wqbuf)

    x = xbuf[...].astype(jnp.float32)
    x = jnp.concatenate([x] * (_ROWS // B), axis=0)
    xn = _layernorm(x).astype(jnp.bfloat16)
    row = jax.lax.broadcasted_iota(jnp.int32, (_ROWS, P), 0)
    col = jax.lax.broadcasted_iota(jnp.int32, (_ROWS, P), 1)
    head = row & (_NH - 1)
    diag = jnp.logical_and(col >= head * Dh, col < (head + 1) * Dh)
    o_scr[...] = jnp.zeros_like(o_scr)
    attn_scr[...] = jnp.zeros_like(attn_scr)

    def step(t):
        s, g = _divmod(t, G)
        j, b = _divmod(_divmod(s, 2)[0], B)
        slot = _divmod(s, _NB)[1]
        past = t + _LAG - n_steps

        @pl.when(past < 0)
        def _():
            issue_cache(t + _LAG)

        @pl.when(past >= 0)
        def _():
            turn = sem.at[_divmod(n_slabs + past, _NB)[1]]

            @pl.when(past >= _NB)
            def _():
                part = past - _NB
                _wait_for(turn, wobuf.at[part])
                done = n_groups - 1
                o = [o_scr[a, :, _block(part, _OW)] for a in range(done)]
                o = jnp.concatenate(o, axis=1).astype(jnp.bfloat16)
                attn_scr[...] += _dot(o, wobuf[part, :done].reshape(done * _OW, D))

            @pl.when(past < NO)
            def _():
                issue_wo(past, turn)

            @pl.when(past >= NO)
            def _():
                issue_gate_up(past - NO, turn)

        @pl.when(g == 0)
        def _():
            _wait_for(sem.at[slot], ring.at[slot])

        def cache():
            return ring[slot, :, :, :, :, :, _block(g, _CW)].reshape(P, _CW)

        @pl.when((s & 1) == 0)
        def _():
            @pl.when(g == 0)
            def _():
                q = _dot(xn, wqbuf[:, :, :, _block(j, P)].reshape(D, P))
                q = jnp.sum(jnp.where(row == b, q, 0.0), axis=0, keepdims=True)
                q_scr[...] = jnp.where(diag, q, 0.0)
                m_scr[...] = jnp.full_like(m_scr, -jnp.inf)

            scores = _dot(q_scr[...].astype(jnp.bfloat16), cache()) * scale
            s_scr[:, _block(g, _CW)] = scores
            m_scr[...] = jnp.maximum(m_scr[...], jnp.max(scores, axis=-1, keepdims=True))

        @pl.when((s & 1) == 1)
        def _():
            @pl.when(g == 0)
            def _():
                l_scr[...] = jnp.zeros_like(l_scr)
                acc_scr[...] = jnp.zeros_like(acc_scr)

            e = jnp.exp(s_scr[:, _block(g, _CW)] - m_scr[...])
            l_scr[...] += jnp.sum(e, axis=-1, keepdims=True)
            acc_scr[...] += _dot_nt(e.astype(jnp.bfloat16), cache())

            @pl.when(g == G - 1)
            def _():
                own = jnp.logical_and(diag, row < _NH)
                o = jnp.where(own, acc_scr[...] / l_scr[...], 0.0)
                o = jnp.sum(o, axis=0, keepdims=True)
                o_scr[j] = jnp.where(row == b, o, o_scr[j])

    _loop(n_steps, step)

    for f in range(1, NF):
        issue_down(f)
    o = o_scr[n_groups - 1].astype(jnp.bfloat16)
    h = x + (attn_scr[...] + _dot(o, wobuf[:, n_groups - 1].reshape(P, D)))
    hn = _layernorm(h)
    hb = hn.astype(jnp.bfloat16)
    r = jnp.sum(hn * wrbuf[...].astype(jnp.float32).reshape(1, D), axis=-1, keepdims=True)
    r_gate = jax.nn.sigmoid(r)
    acts = []
    for f in range(NF):
        _wait_for(sem.at[(n_slabs + NO + f) % _NB], wgbuf.at[f], wubuf.at[f])
        gate = _dot(hb, wgbuf[f])
        acts.append((gate * jax.nn.sigmoid(gate) * _dot(hb, wubuf[f])).astype(jnp.bfloat16))
    y = jnp.zeros((_ROWS, D), jnp.float32)
    for f in range(NF):
        _wait_for(sem.at[_NB + f], wdbuf.at[f])
        y = y + _dot(acts[f], wdbuf[f])
    out = h + (hn + (hn * 0.0 + y * r_gate))
    out_ref[...] = out[:B].astype(out_ref.dtype)


@jax.jit
def pallas_sequential_preLN__mha_block_cached__moe_arch_mod__decode_kernel(
    A_x: jax.Array,
    A_k_cache: jax.Array,
    A_v_cache: jax.Array,
    A_wq: jax.Array,
    A_wo: jax.Array,
    B_x: jax.Array,
    B_w_r: jax.Array,
    B_w_gate: jax.Array,
    B_w_up: jax.Array,
    B_w_down: jax.Array,
):
    del B_x
    B, Sq, D = A_x.shape
    _, H, Sk, Dh = A_k_cache.shape
    F = B_w_gate.shape[1]
    P = _NH * Dh
    assert (B, Sq, D, H, Sk, Dh, F) == (4, 1, 640, 32, 8192, 192, 1536)
    assert _LAG == P // _OW + F // _FW and F // _FW == _NB
    dt = A_k_cache.dtype
    f32 = jnp.float32

    slab = (P // _SR // 4, 2, 2, _SR // _ROWS, _ROWS, Sk)
    kt = jnp.swapaxes(A_k_cache, 2, 3).reshape(B * H // _NH, *slab)
    vt = jnp.swapaxes(A_v_cache, 2, 3).reshape(B * H // _NH, *slab)
    wq = A_wq.reshape(D // _SR, _SR // _ROWS, _ROWS, H * Dh)

    out = pl.pallas_call(
        functools.partial(_body, B=B, H=H, Dh=Dh, Sk=Sk, D=D, F=F),
        in_specs=[pl.BlockSpec(memory_space=pl.ANY)] * 9,
        out_specs=pl.BlockSpec(memory_space=pltpu.VMEM),
        out_shape=jax.ShapeDtypeStruct((B, D), A_x.dtype),
        scratch_shapes=[
            pltpu.VMEM((_NB, *slab), dt),
            pltpu.VMEM(wq.shape, dt),
            pltpu.VMEM((P // _OW, H // _NH, _OW, D), dt),
            pltpu.VMEM((F // _FW, D, _FW), dt),
            pltpu.VMEM((F // _FW, D, _FW), dt),
            pltpu.VMEM((F // _FW, _FW, D), dt),
            pltpu.VMEM((B, D), dt),
            pltpu.VMEM((D,), dt),
            pltpu.VMEM((_ROWS, P), f32),
            pltpu.VMEM((_ROWS, Sk), f32),
            pltpu.VMEM((_ROWS, 1), f32),
            pltpu.VMEM((_ROWS, 1), f32),
            pltpu.VMEM((_ROWS, P), f32),
            pltpu.VMEM((H // _NH, _ROWS, P), f32),
            pltpu.VMEM((_ROWS, D), f32),
            pltpu.SemaphoreType.DMA((_NB + F // _FW,)),
        ],
        compiler_params=pltpu.CompilerParams(vmem_limit_bytes=80 * 1024 * 1024),
    )(A_x.reshape(B, D), kt, vt, wq, A_wo, B_w_r, B_w_gate, B_w_up, B_w_down)
    return out.reshape(B, Sq, D)
```

```python
import functools

import jax
import jax.numpy as jnp
import jax.experimental.pallas as pl
import jax.experimental.pallas.tpu as pltpu

_EPS = 1e-5
_ROWS = 8
_NH = 4
_SR = 64
_CW = 1024
_NB = 3
_LAG = 9
_SKEW = 2
_OW = 128
_FW = 512


def _layernorm(x):
    m = jnp.mean(x, axis=-1, keepdims=True)
    d = x - m
    v = jnp.mean(d * d, axis=-1, keepdims=True)
    return d / jnp.sqrt(v + _EPS)


def _dot(a, b):
    return jnp.dot(a, b, preferred_element_type=jnp.float32)


def _dot_nt(a, b):
    return jax.lax.dot_general(
        a, b, (((1,), (1,)), ((), ())), preferred_element_type=jnp.float32
    )


def _wait_for(sem, buf):
    pltpu.make_async_copy(buf, buf, sem).wait()


def _loop(n, fn):
    jax.lax.fori_loop(0, n, lambda i, carry: fn(i), None)


def _divmod(i, n):
    if n & (n - 1) == 0:
        return jax.lax.shift_right_logical(i, n.bit_length() - 1), i & (n - 1)
    return jax.lax.div(i, n), jax.lax.rem(i, n)


def _span(start, size, align):
    return pl.ds(start if isinstance(start, int) else pl.multiple_of(start, align), size)


def _block(i, size):
    return _span(i * size, size, size)


def _body(
    x_hbm, kt_hbm, vt_hbm, wq_hbm, wo_hbm, wr_hbm, wg_hbm, wu_hbm, wd_hbm,
    out_ref,
    ring, wqbuf, wobuf, wgubuf, wdbuf, xbuf, wrbuf,
    q_scr, s_scr, m_scr, l_scr, acc_scr, o_scr, attn_scr, sem,
    *, B, H, Dh, Sk, D, F,
):
    P = _NH * Dh
    n_groups = H // _NH
    G = Sk // _CW
    pairs = P // _SR // 4
    n_slabs = 2 * n_groups * B
    n_steps = n_slabs * G
    NO = P // _OW
    NF = F // _FW
    scale = Dh ** -0.5

    def row_tile(t):
        s, r = _divmod(t, G)
        j, b = _divmod(_divmod(s, 2)[0], B)
        return b * n_groups + j, _divmod(s, _NB)[1], r, s

    def start_runs(hbm, tile, c, f, queue):
        n, slot, r, _ = tile
        at = (f, slice(None), queue, r, slice(None), _block(c, _CW))
        pltpu.make_async_copy(
            hbm.at[(n, *at)], ring.at[(slot, *at)], sem.at[slot]
        ).start(priority=queue)

    def with_cache(tile, fn):
        s = tile[-1]
        for i, hbm in enumerate((kt_hbm, vt_hbm)):
            pl.when(jnp.logical_and((s & 1) == i, s < n_slabs))(functools.partial(fn, hbm))

    def issue_cache(t):
        first, second, third = row_tile(t), row_tile(t + 1), row_tile(t + 2)

        def both(hbm0, hbm1):
            def column(c):
                for f in range(pairs):
                    start_runs(hbm0, first, c, f, 0)
                    carry, f1 = divmod(f + _SKEW, pairs)
                    start_runs(hbm1, second, c + carry, f1, 1)

            _loop(G - 1, column)
            for f in range(pairs):
                start_runs(hbm0, first, G - 1, f, 0)
                carry, f1 = divmod(f + _SKEW, pairs)
                if carry:
                    with_cache(third, lambda hbm: start_runs(hbm, third, 0, f1, 1))
                else:
                    start_runs(hbm1, second, G - 1, f1, 1)

        @pl.when(t + 1 < n_steps)
        def _():
            with_cache(first, lambda hbm0: with_cache(second, functools.partial(both, hbm0)))

        @pl.when(t + 1 == n_steps)
        def _():
            def column(c):
                for f, (r0, size) in enumerate(((0, 24), (24, 24), (48, 16))):
                    start_runs(vt_hbm, first, c, f, 0)
                    rows = _span(c * (_FW // G) + r0, size, _ROWS)
                    pltpu.make_async_copy(
                        wd_hbm.at[rows, :], wdbuf.at[0, rows, :], sem.at[_NB]
                    ).start(priority=1)

            _loop(G, column)

    def start_wq(f, r, c, queue):
        at = (f, r, slice(None), _block(c, H * Dh // pairs))
        pltpu.make_async_copy(wq_hbm.at[at], wqbuf.at[at], sem.at[_NB - 1]).start(priority=queue)

    def issue_wq(i):
        n = D // _SR - 1
        for h in range(2):
            for c in range(pairs):
                for f in range(n):
                    start_wq(f, 2 * i + h, c, ((h * pairs + c) * n + f) % 2)

    def head_start(c):
        for f in range(pairs):
            start_wq(D // _SR - 1, c, f, 0)
            start_runs(kt_hbm, (0, 0, 0, 0), c, f, 1)

    def issue_wo(part, s):
        def piece(i):
            for j in range(n_groups):
                pltpu.make_async_copy(
                    wo_hbm.at[_span(j * P + part * _OW + i * 32, 32, 32), :],
                    wobuf.at[part, j, _block(i, 32), :],
                    s,
                ).start(priority=j % 2)

        _loop(_OW // 32, piece)

    def issue_gate_up(f, s):
        def piece(i):
            for r0 in range(0, D, D // 4):
                rows = _span(r0 + i * 32, 32, 32)
                for queue, hbm in enumerate((wg_hbm, wu_hbm)):
                    pltpu.make_async_copy(
                        hbm.at[rows, _block(f, _FW)], wgubuf.at[f, queue, rows, :], s
                    ).start(priority=queue)

        _loop(D // 4 // 32, piece)

    def issue_down(f):
        def piece(i):
            for a, r0 in enumerate(range(0, _FW, _FW // 4)):
                pltpu.make_async_copy(
                    wd_hbm.at[_span(f * _FW + r0 + i * 16, 16, 16), :],
                    wdbuf.at[f, _span(r0 + i * 16, 16, 16), :],
                    sem.at[_NB + f],
                ).start(priority=a % 2)

        _loop(_FW // 4 // 16, piece)

    x_copy = pltpu.make_async_copy(x_hbm, xbuf, sem.at[_NB])
    wr_copy = pltpu.make_async_copy(wr_hbm, wrbuf, sem.at[_NB + 1])
    x_copy.start()
    wr_copy.start(priority=1)
    _loop(_SR // _ROWS // 2, issue_wq)
    _loop(G, head_start)
    for f in range(_SKEW):
        start_runs(kt_hbm, (0, 0, 1, 0), 0, f, 1)
    _loop(_LAG, issue_cache)
    x_copy.wait()
    wr_copy.wait()
    _wait_for(sem.at[_NB - 1], wqbuf)

    x = xbuf[...].astype(jnp.float32)
    x = jnp.concatenate([x] * (_ROWS // B), axis=0)
    xn = _layernorm(x).astype(jnp.bfloat16)
    row = jax.lax.broadcasted_iota(jnp.int32, (_ROWS, P), 0)
    col = jax.lax.broadcasted_iota(jnp.int32, (_ROWS, P), 1)
    head = row & (_NH - 1)
    diag = jnp.logical_and(col >= head * Dh, col < (head + 1) * Dh)
    o_scr[...] = jnp.zeros_like(o_scr)
    attn_scr[...] = jnp.zeros_like(attn_scr)

    def step(t):
        s, g = _divmod(t, G)
        j, b = _divmod(_divmod(s, 2)[0], B)
        slot = _divmod(s, _NB)[1]
        past = t + _LAG - n_steps

        @pl.when(past < 0)
        def _():
            issue_cache(t + _LAG)

        @pl.when(past >= 0)
        def _():
            turn = sem.at[_divmod(n_slabs + past, _NB)[1]]

            @pl.when(past >= _NB)
            def _():
                part = past - _NB
                _wait_for(turn, wobuf.at[part])
                done = n_groups - 1
                o = [o_scr[a, :, _block(part, _OW)] for a in range(done)]
                o = jnp.concatenate(o, axis=1).astype(jnp.bfloat16)
                attn_scr[...] += _dot(o, wobuf[part, :done].reshape(done * _OW, D))

            @pl.when(past < NO)
            def _():
                issue_wo(past, turn)

            @pl.when(past >= NO)
            def _():
                issue_gate_up(past - NO, turn)

        @pl.when(g == 0)
        def _():
            _wait_for(sem.at[slot], ring.at[slot])

        def cache():
            return ring[slot, :, :, :, :, :, _block(g, _CW)].reshape(P, _CW)

        @pl.when((s & 1) == 0)
        def _():
            @pl.when(g == 0)
            def _():
                q = _dot(xn, wqbuf[:, :, :, _block(j, P)].reshape(D, P))
                q = jnp.sum(jnp.where(row == b, q, 0.0), axis=0, keepdims=True)
                q_scr[...] = jnp.where(diag, q, 0.0)
                m_scr[...] = jnp.full_like(m_scr, -jnp.inf)

            scores = _dot(q_scr[...].astype(jnp.bfloat16), cache()) * scale
            s_scr[:, _block(g, _CW)] = scores
            m_scr[...] = jnp.maximum(m_scr[...], jnp.max(scores, axis=-1, keepdims=True))

        @pl.when((s & 1) == 1)
        def _():
            @pl.when(g == 0)
            def _():
                l_scr[...] = jnp.zeros_like(l_scr)
                acc_scr[...] = jnp.zeros_like(acc_scr)

            e = jnp.exp(s_scr[:, _block(g, _CW)] - m_scr[...])
            l_scr[...] += jnp.sum(e, axis=-1, keepdims=True)
            acc_scr[...] += _dot_nt(e.astype(jnp.bfloat16), cache())

            @pl.when(g == G - 1)
            def _():
                own = jnp.logical_and(diag, row < _NH)
                o = jnp.where(own, acc_scr[...] / l_scr[...], 0.0)
                o = jnp.sum(o, axis=0, keepdims=True)
                o_scr[j] = jnp.where(row == b, o, o_scr[j])

    _loop(n_steps, step)

    for f in range(1, NF):
        issue_down(f)
    o = o_scr[n_groups - 1].astype(jnp.bfloat16)
    h = x + (attn_scr[...] + _dot(o, wobuf[:, n_groups - 1].reshape(P, D)))
    hn = _layernorm(h)
    hb = hn.astype(jnp.bfloat16)
    r = jnp.sum(hn * wrbuf[...].astype(jnp.float32).reshape(1, D), axis=-1, keepdims=True)
    r_gate = jax.nn.sigmoid(r)
    acts = []
    for f in range(NF):
        _wait_for(sem.at[(n_slabs + NO + f) % _NB], wgubuf.at[f])
        gate = _dot(hb, wgubuf[f, 0])
        acts.append((gate * jax.nn.sigmoid(gate) * _dot(hb, wgubuf[f, 1])).astype(jnp.bfloat16))
    y = jnp.zeros((_ROWS, D), jnp.float32)
    for f in range(NF):
        _wait_for(sem.at[_NB + f], wdbuf.at[f])
        y = y + _dot(acts[f], wdbuf[f])
    out = h + (hn + (hn * 0.0 + y * r_gate))
    out_ref[...] = out[:B].astype(out_ref.dtype)


@jax.jit
def pallas_sequential_preLN__mha_block_cached__moe_arch_mod__decode_kernel(
    A_x: jax.Array,
    A_k_cache: jax.Array,
    A_v_cache: jax.Array,
    A_wq: jax.Array,
    A_wo: jax.Array,
    B_x: jax.Array,
    B_w_r: jax.Array,
    B_w_gate: jax.Array,
    B_w_up: jax.Array,
    B_w_down: jax.Array,
):
    del B_x
    B, Sq, D = A_x.shape
    _, H, Sk, Dh = A_k_cache.shape
    F = B_w_gate.shape[1]
    P = _NH * Dh
    assert (B, Sq, D, H, Sk, Dh, F) == (4, 1, 640, 32, 8192, 192, 1536)
    assert _LAG == P // _OW + F // _FW and F // _FW == _NB
    dt = A_k_cache.dtype
    f32 = jnp.float32

    slab = (P // _SR // 4, 2, 2, _SR // _ROWS, _ROWS, Sk)
    kt = jnp.swapaxes(A_k_cache, 2, 3).reshape(B * H // _NH, *slab)
    vt = jnp.swapaxes(A_v_cache, 2, 3).reshape(B * H // _NH, *slab)
    wq = A_wq.reshape(D // _SR, _SR // _ROWS, _ROWS, H * Dh)

    out = pl.pallas_call(
        functools.partial(_body, B=B, H=H, Dh=Dh, Sk=Sk, D=D, F=F),
        in_specs=[pl.BlockSpec(memory_space=pl.ANY)] * 9,
        out_specs=pl.BlockSpec(memory_space=pltpu.VMEM),
        out_shape=jax.ShapeDtypeStruct((B, D), A_x.dtype),
        scratch_shapes=[
            pltpu.VMEM((_NB, *slab), dt),
            pltpu.VMEM(wq.shape, dt),
            pltpu.VMEM((P // _OW, H // _NH, _OW, D), dt),
            pltpu.VMEM((F // _FW, 2, D, _FW), dt),
            pltpu.VMEM((F // _FW, _FW, D), dt),
            pltpu.VMEM((B, D), dt),
            pltpu.VMEM((D,), dt),
            pltpu.VMEM((_ROWS, P), f32),
            pltpu.VMEM((_ROWS, Sk), f32),
            pltpu.VMEM((_ROWS, 1), f32),
            pltpu.VMEM((_ROWS, 1), f32),
            pltpu.VMEM((_ROWS, P), f32),
            pltpu.VMEM((H // _NH, _ROWS, P), f32),
            pltpu.VMEM((_ROWS, D), f32),
            pltpu.SemaphoreType.DMA((_NB + F // _FW,)),
        ],
        compiler_params=pltpu.CompilerParams(vmem_limit_bytes=80 * 1024 * 1024),
    )(A_x.reshape(B, D), kt, vt, wq, A_wo, B_w_r, B_w_gate, B_w_up, B_w_down)
    return out.reshape(B, Sq, D)
```
